```python
import jax
import jax.numpy as jnp

def _softmax(x, axis=-1):
    return jax.nn.softmax(x, axis=axis)
def _gelu(x):
    return jax.nn.gelu(x, approximate=True)
def _silu(x):
    return jax.nn.silu(x)
def _sigmoid(x):
    return jax.nn.sigmoid(x)
def _layernorm(x, axis=-1, eps=1e-5):
    m = jnp.mean(x, axis=axis, keepdims=True)
    v = jnp.var(x, axis=axis, keepdims=True)
    return (x - m) / jnp.sqrt(v + eps)
def _scatter_add(tgt, idx, src, axis=0):
    return tgt.at[idx].add(src)
def _segment_sum(src, seg, n):
    return jax.ops.segment_sum(src, seg, n)
class _Rng:
    def __init__(self, key):
        self._k = key
    def _next(self):
        self._k, sub = jax.random.split(self._k)
        return sub
    def normal(self, shape):
        return jax.random.normal(self._next(), shape, dtype=jnp.bfloat16)
    def randint(self, lo, hi, shape):
        return jax.random.randint(self._next(), shape, lo, hi, dtype=jnp.int32)
    def uniform(self, shape, lo=0.0, hi=1.0):
        return jax.random.uniform(self._next(), shape, jnp.bfloat16, lo, hi)
    def permutation(self, n):
        return jax.random.permutation(self._next(), n)


kernel_name = 'sequential_preLN__mha_block_cached__moe_arch_mod__decode'

def setup_inputs():
    _rng = _Rng(jax.random.key(int.from_bytes(__import__("os").urandom(4), "little")))
    _w = (lambda a: (lambda t: t.astype(jnp.bfloat16) if jnp.issubdtype(t.dtype, jnp.floating) else t)(jnp.asarray(a)))
    def _A_setup():
        B, Sq, D = 4, 1, 640
        H, Sk, Dh = 32, 8192, 192
        return {
            "x": _w((lambda *s: _rng.normal(s) * 0.05)(B, Sq, D)),
            "k_cache": _w((lambda *s: _rng.normal(s) * 0.05)(B, H, Sk, Dh)),
            "v_cache": _w((lambda *s: _rng.normal(s) * 0.05)(B, H, Sk, Dh)),
            "wq": _w((lambda *s: _rng.normal(s) * 0.05)(D, H * Dh) * (D ** -0.5)),
            "wo": _w((lambda *s: _rng.normal(s) * 0.05)(H * Dh, D) * ((H * Dh) ** -0.5)),
        }
    _A_in = _A_setup()

    def _B_setup():
        B, S, D, F, C = 4, 1, 640, 1536, 1
        return {
            "x": _w((lambda *s: _rng.normal(s) * 0.05)(B, S, D)),
            "w_r": _w((lambda *s: _rng.normal(s) * 0.05)(D)),
            "w_gate": _w((lambda *s: _rng.normal(s) * 0.05)(D, F)),
            "w_up": _w((lambda *s: _rng.normal(s) * 0.05)(D, F)),
            "w_down": _w((lambda *s: _rng.normal(s) * 0.05)(F, D)),
        }
    _B_in = _B_setup()

    return {
        "A_x": _A_in["x"],
        "A_k_cache": _A_in["k_cache"],
        "A_v_cache": _A_in["v_cache"],
        "A_wq": _A_in["wq"],
        "A_wo": _A_in["wo"],
        "B_x": _B_in["x"],
        "B_w_r": _B_in["w_r"],
        "B_w_gate": _B_in["w_gate"],
        "B_w_up": _B_in["w_up"],
        "B_w_down": _B_in["w_down"],
    }

def reference(A_x, A_k_cache, A_v_cache, A_wq, A_wo, B_x, B_w_r, B_w_gate, B_w_up, B_w_down):
    def _A_ref(x, k_cache, v_cache, wq, wo):
        B, Sq, D = x.shape
        H, Dh = 32, 192
        q = (lambda x, *d: x.transpose(*d))((x @ wq).reshape(B, Sq, H, Dh), 0, 2, 1, 3)
        scores = jnp.einsum("bhqd,bhkd->bhqk", q, k_cache) * (Dh ** -0.5)
        p = _softmax(scores, axis=-1)
        o = jnp.einsum("bhqk,bhkd->bhqd", p, v_cache)
        return (lambda x, *d: x.transpose(*d))(o, 0, 2, 1, 3).reshape(B, Sq, H * Dh) @ wo

    def _B_ref(x, w_r, w_gate, w_up, w_down):
        B, S, D = x.shape
        C = 1
        r = x @ w_r
        idx = jnp.argsort(-r, axis=-1)[:, :C]
        idx_e = jnp.repeat(idx.reshape(B, C, 1), D, axis=2)
        x_sel = jnp.take_along_axis(x, idx_e, axis=1)
        g = _silu(x_sel @ w_gate)
        u = x_sel @ w_up
        y = (g * u) @ w_down
        r_sel = _sigmoid(jnp.take_along_axis(r, idx, axis=1))
        y = y * r_sel.reshape(B, C, 1)
        b_off = (jnp.arange(B) * S).reshape(B, 1)
        flat_idx = (idx + b_off).reshape(B * C)
        zero = (x * 0.0).reshape(B * S, D)
        upd = _scatter_add(zero, flat_idx, y.reshape(B * C, D), axis=0)
        return x + upd.reshape(B, S, D)

    x = A_x
    h = x + _A_ref(_layernorm(x, axis=-1), A_k_cache, A_v_cache, A_wq, A_wo)
    h2 = h + _B_ref(_layernorm(h, axis=-1), B_w_r, B_w_gate, B_w_up, B_w_down)
    return h2
```

```python
import jax
import jax.numpy as jnp
from jax import lax
import jax.experimental.pallas as pl
import jax.experimental.pallas.tpu as pltpu

_NBUF = 4
_CR = 16
_CC = 4096
_NSPLIT = 8
_EPS = 1e-5


def _layernorm(x):
    m = jnp.mean(x, axis=-1, keepdims=True)
    xc = x - m
    v = jnp.mean(xc * xc, axis=-1, keepdims=True)
    return xc / jnp.sqrt(v + _EPS)


@jax.jit
def pallas_sequential_preLN__mha_block_cached__moe_arch_mod__decode_kernel(
    A_x: jax.Array,
    A_k_cache: jax.Array,
    A_v_cache: jax.Array,
    A_wq: jax.Array,
    A_wo: jax.Array,
    B_x: jax.Array,
    B_w_r: jax.Array,
    B_w_gate: jax.Array,
    B_w_up: jax.Array,
    B_w_down: jax.Array,
):
    B, _, D = A_x.shape
    _, H, S, DH = A_k_cache.shape
    F = B_w_gate.shape[1]
    PR = 2 * DH
    NP = H // 2
    chunks = [(r, c) for r in range(0, PR, _CR) for c in range(0, S, _CC)]
    NCH = len(chunks)
    CPS = NCH // _NSPLIT
    SC = S // _NSPLIT

    def kernel(x_ref, wr_ref, k_hbm, v_hbm, wq_hbm, wo_hbm, wg_hbm, wu_hbm, wd_hbm, o_ref,
               kv, wq_v, wo_v, wg_v, wu_v, wd_v, q_s, o_s, sems, wsems):

        def start_chunks(src, pair, slot, lo, hi):
            r0 = pl.multiple_of(pair * PR, PR)
            for i in range(lo, hi):
                r, c = chunks[i]
                pltpu.make_async_copy(
                    src.at[pl.ds(r0 + r, _CR), pl.ds(c, _CC)],
                    kv.at[slot, pl.ds(r, _CR), pl.ds(c, _CC)],
                    sems.at[slot]).start(priority=i % 2)

        def wait_unit(slot):
            pltpu.make_async_copy(kv.at[slot], kv.at[slot], sems.at[slot]).wait()

        def wcopy(i):
            src, dst = ((wq_hbm, wq_v), (wo_hbm, wo_v), (wg_hbm, wg_v),
                        (wu_hbm, wu_v), (wd_hbm, wd_v))[i]
            return pltpu.make_async_copy(src, dst, wsems.at[i])

        wcopy(0).start()
        start_chunks(k_hbm, 0, 0, 0, NCH)
        start_chunks(v_hbm, 0, 1, 0, NCH)

        x = x_ref[...].astype(jnp.float32)
        xn = _layernorm(x).astype(jnp.bfloat16)
        xn8 = jnp.concatenate([xn, jnp.zeros((8 - B, D), jnp.bfloat16)], axis=0)
        o_s[...] = jnp.zeros(o_s.shape, o_s.dtype)
        wcopy(0).wait()
        for p in range(NP):
            q_s[p] = jnp.dot(xn8, wq_v[:, p * PR:(p + 1) * PR],
                             preferred_element_type=jnp.float32)

        row = lax.broadcasted_iota(jnp.int32, (8, PR), 0)
        col = lax.broadcasted_iota(jnp.int32, (8, PR), 1)
        qmask = jnp.logical_or(jnp.logical_and(row == 0, col < DH),
                               jnp.logical_and(row == 1, col >= DH))
        scale = DH ** -0.5

        def pair_body(p, last):
            b = p // NP
            hp = p % NP
            ks = (2 * p) % _NBUF
            vs = (2 * p + 1) % _NBUF
            nks = (2 * p + 2) % _NBUF
            nvs = (2 * p + 3) % _NBUF
            qrow = q_s[hp, pl.ds(b, 1), :]
            qblk = jnp.where(qmask, jnp.broadcast_to(qrow, (8, PR)), 0.0).astype(jnp.bfloat16)
            wait_unit(ks)
            s_parts = []
            for j in range(_NSPLIT):
                if not last:
                    start_chunks(k_hbm, p + 1, nks, j * CPS, (j + 1) * CPS)
                s_parts.append(jnp.dot(qblk, kv[ks, :, j * SC:(j + 1) * SC],
                                       preferred_element_type=jnp.float32) * scale)
            m = s_parts[0]
            for sp in s_parts[1:]:
                m = jnp.maximum(m, sp)
            m = jnp.max(m, axis=-1, keepdims=True)
            wait_unit(vs)
            acc = jnp.zeros((8, PR), jnp.float32)
            l = jnp.zeros((8, SC), jnp.float32)
            for j in range(_NSPLIT):
                if not last:
                    start_chunks(v_hbm, p + 1, nvs, j * CPS, (j + 1) * CPS)
                e = jnp.exp(s_parts[j] - m)
                l = l + e
                acc = acc + lax.dot_general(
                    e.astype(jnp.bfloat16), kv[vs, :, j * SC:(j + 1) * SC],
                    (((1,), (1,)), ((), ())), preferred_element_type=jnp.float32)
            l = jnp.sum(l, axis=-1, keepdims=True)
            on = jnp.where(qmask, acc / l, 0.0)
            o_s[hp, pl.ds(b, 1), :] = jnp.sum(on, axis=0, keepdims=True)

        def loop_body(p, c):
            pair_body(p, False)
            return c

        lax.fori_loop(0, B * NP - 1, loop_body, 0)
        for i in range(1, 5):
            wcopy(i).start()
        pair_body(B * NP - 1, True)

        wcopy(1).wait()
        attn = jnp.zeros((8, D), jnp.float32)
        for p in range(NP):
            attn = attn + jnp.dot(o_s[p].astype(jnp.bfloat16), wo_v[p * PR:(p + 1) * PR, :],
                                  preferred_element_type=jnp.float32)
        h = x + attn[:B]
        hn = _layernorm(h)
        hb = hn.astype(jnp.bfloat16)
        r = jnp.sum(hn * wr_ref[...].astype(jnp.float32).reshape(1, D), axis=-1, keepdims=True)
        hb8 = jnp.concatenate([hb, jnp.zeros((8 - B, D), jnp.bfloat16)], axis=0)
        wcopy(2).wait()
        g = jnp.dot(hb8, wg_v[...], preferred_element_type=jnp.float32)
        g = g * jax.nn.sigmoid(g)
        wcopy(3).wait()
        u = jnp.dot(hb8, wu_v[...], preferred_element_type=jnp.float32)
        gu = (g * u).astype(jnp.bfloat16)
        wcopy(4).wait()
        y = jnp.dot(gu, wd_v[...], preferred_element_type=jnp.float32)[:B]
        y = y * jax.nn.sigmoid(r)
        o_ref[...] = (h + (hn + (hn * 0.0 + y))).astype(o_ref.dtype)

    kt = jnp.transpose(A_k_cache, (0, 1, 3, 2)).reshape(B * H * DH, S)
    vt = jnp.transpose(A_v_cache, (0, 1, 3, 2)).reshape(B * H * DH, S)
    vm = pl.BlockSpec(memory_space=pltpu.VMEM)
    hbm = pl.BlockSpec(memory_space=pl.ANY)
    out = pl.pallas_call(
        kernel,
        in_specs=[vm, vm] + [hbm] * 7,
        out_specs=vm,
        out_shape=jax.ShapeDtypeStruct((B, D), jnp.bfloat16),
        scratch_shapes=[
            pltpu.VMEM((_NBUF, PR, S), jnp.bfloat16),
            pltpu.VMEM((D, H * DH), jnp.bfloat16),
            pltpu.VMEM((H * DH, D), jnp.bfloat16),
            pltpu.VMEM((D, F), jnp.bfloat16),
            pltpu.VMEM((D, F), jnp.bfloat16),
            pltpu.VMEM((F, D), jnp.bfloat16),
            pltpu.VMEM((NP, 8, PR), jnp.float32),
            pltpu.VMEM((NP, 8, PR), jnp.float32),
            pltpu.SemaphoreType.DMA((_NBUF,)),
            pltpu.SemaphoreType.DMA((5,)),
        ],
        compiler_params=pltpu.CompilerParams(vmem_limit_bytes=100 * 1024 * 1024),
    )(A_x.reshape(B, D), B_w_r, kt, vt, A_wq, A_wo, B_w_gate, B_w_up, B_w_down)
    return out.reshape(B, 1, D)
```

```python
import jax
import jax.numpy as jnp
from jax import lax
import jax.experimental.pallas as pl
import jax.experimental.pallas.tpu as pltpu

_NBUF = 3
_CR, _CC = 96, 256
_EPS = 1e-5


def _layernorm(x):
    m = jnp.mean(x, axis=-1, keepdims=True)
    xc = x - m
    v = jnp.mean(xc * xc, axis=-1, keepdims=True)
    return xc / jnp.sqrt(v + _EPS)


def _loop(n, fn):
    def body(j, carry):
        fn(j)
        return carry
    lax.fori_loop(0, n, body, 0)


@jax.jit
def pallas_sequential_preLN__mha_block_cached__moe_arch_mod__decode_kernel(
    A_x: jax.Array,
    A_k_cache: jax.Array,
    A_v_cache: jax.Array,
    A_wq: jax.Array,
    A_wo: jax.Array,
    B_x: jax.Array,
    B_w_r: jax.Array,
    B_w_gate: jax.Array,
    B_w_up: jax.Array,
    B_w_down: jax.Array,
):
    del B_x
    B, Sq, D = A_x.shape
    _, H, S, DH = A_k_cache.shape
    F = B_w_gate.shape[1]
    PR = 2 * DH
    NP = H // 2
    SC = 2 * _CC
    NJ = S // SC
    NF = F // PR
    assert Sq == 1 and B <= 8 and NJ == NP and 3 * NF <= NJ
    bf16, f32 = jnp.bfloat16, jnp.float32

    def kernel(x_hbm, wr_hbm, k_hbm, v_hbm, wq_hbm, wo_hbm, wg_hbm, wu_hbm, wd_hbm, o_ref,
               kv, x_v, wr_v, wq_v, wo_v, wg_v, wu_v, wd_v, q_s, o_s, s_s, kv_sems, w_sems):
        WQ, WO, WG, WU, WD, X, WR = range(7)
        pairs = ((wq_hbm, wq_v), (wo_hbm, wo_v), (wg_hbm, wg_v), (wu_hbm, wu_v),
                 (wd_hbm, wd_v), (x_hbm, x_v), (wr_hbm, wr_v))

        def start_kv(src, pair, slot, j):
            r0 = pl.multiple_of(pair * PR, PR)
            c0 = pl.multiple_of(j * SC, SC)
            for r in range(0, PR, _CR):
                for t in range(2):
                    pltpu.make_async_copy(
                        src.at[pl.ds(r0 + r, _CR), pl.ds(c0 + t * _CC, _CC)],
                        kv.at[slot, j, pl.ds(r, _CR), pl.ds(t * _CC, _CC)],
                        kv_sems.at[slot]).start(priority=t)

        def wait_kv(slot):
            pltpu.make_async_copy(kv.at[slot], kv.at[slot], kv_sems.at[slot]).wait()

        def whole(i):
            return pltpu.make_async_copy(pairs[i][0], pairs[i][1], w_sems.at[i])

        def start_pieces(i, pieces):
            for n, sl in enumerate(pieces):
                pltpu.make_async_copy(pairs[i][0].at[sl], pairs[i][1].at[sl],
                                      w_sems.at[i]).start(priority=n % 2)

        def start_cols(i, g):
            c0 = pl.multiple_of(g * PR, PR)
            start_pieces(i, [(pl.ds(r, 64), pl.ds(c0, PR)) for r in range(0, D, 64)])

        def start_rows(i, g):
            r0 = pl.multiple_of(g * PR, PR)
            start_pieces(i, [(pl.ds(r0 + r, DH), pl.ds(c, 128))
                             for c in range(0, D, 128) for r in range(0, PR, DH)])

        def pad8(a):
            return jnp.concatenate([a, jnp.zeros((8 - B, D), a.dtype)], axis=0)

        whole(X).start()
        whole(WR).start(priority=1)
        _loop(NP, lambda g: start_cols(WQ, g))
        _loop(NJ, lambda j: start_kv(k_hbm, 0, 0, j))
        whole(X).wait()
        whole(WR).wait()
        xn = pad8(_layernorm(x_v[...].astype(f32)).astype(bf16))
        o_s[...] = jnp.zeros(o_s.shape, f32)
        whole(WQ).wait()

        def q_step(g):
            start_kv(v_hbm, 0, 1, g)
            w = wq_v[:, pl.ds(pl.multiple_of(g * PR, PR), PR)]
            q_s[g] = jnp.dot(xn, w, preferred_element_type=f32)
        _loop(NP, q_step)

        row = lax.broadcasted_iota(jnp.int32, (8, PR), 0)
        col = lax.broadcasted_iota(jnp.int32, (8, PR), 1)
        own = jnp.logical_or(jnp.logical_and(row == 0, col < DH),
                             jnp.logical_and(row == 1, col >= DH))
        scale = DH ** -0.5

        def attend(p, issue_in_qk, issue_in_pv):
            b, hp = p // NP, p % NP
            ks, vs = (2 * p) % _NBUF, (2 * p + 1) % _NBUF
            q = jnp.broadcast_to(q_s[hp, pl.ds(b, 1), :], (8, PR))
            q = jnp.where(own, q, 0.0).astype(bf16)

            def qk(j, m):
                issue_in_qk(j)
                s = jnp.dot(q, kv[ks, j], preferred_element_type=f32) * scale
                s_s[j] = s
                return jnp.maximum(m, s)

            wait_kv(ks)
            m = lax.fori_loop(0, NJ, qk, jnp.full((8, SC), -jnp.inf, f32))
            m = jnp.max(m, axis=-1, keepdims=True)

            def pv(j, carry):
                acc, l = carry
                issue_in_pv(j)
                e = jnp.exp(s_s[j] - m)
                acc = acc + lax.dot_general(e.astype(bf16), kv[vs, j], (((1,), (1,)), ((), ())),
                                            preferred_element_type=f32)
                return acc, l + e

            wait_kv(vs)
            acc, l = lax.fori_loop(0, NJ, pv, (jnp.zeros((8, PR), f32), jnp.zeros((8, SC), f32)))
            o = jnp.where(own, acc / jnp.sum(l, axis=-1, keepdims=True), 0.0)
            o_s[hp, pl.ds(b, 1), :] = jnp.sum(o, axis=0, keepdims=True)

        _loop(B * NP - 1, lambda p: attend(
            p,
            lambda j: start_kv(k_hbm, p + 1, (2 * p + 2) % _NBUF, j),
            lambda j: start_kv(v_hbm, p + 1, (2 * p + 3) % _NBUF, j)))

        def start_ffn(j):
            pl.when(j < NF)(lambda: start_cols(WG, j))
            pl.when(jnp.logical_and(j >= NF, j < 2 * NF))(lambda: start_cols(WU, j - NF))
            pl.when(jnp.logical_and(j >= 2 * NF, j < 3 * NF))(lambda: start_rows(WD, j - 2 * NF))

        attend(B * NP - 1, lambda j: start_rows(WO, j), start_ffn)

        whole(WO).wait()
        attn = jnp.zeros((8, D), f32)
        for g in range(NP):
            attn = attn + jnp.dot(o_s[g].astype(bf16), wo_v[g * PR:(g + 1) * PR, :],
                                  preferred_element_type=f32)
        h = x_v[...].astype(f32) + attn[:B]
        hn = _layernorm(h)
        r = jnp.sum(hn * wr_v[...].astype(f32).reshape(1, D), axis=-1, keepdims=True)
        hb = pad8(hn.astype(bf16))
        whole(WG).wait()
        gate = jnp.dot(hb, wg_v[...], preferred_element_type=f32)
        gate = gate * jax.nn.sigmoid(gate)
        whole(WU).wait()
        up = jnp.dot(hb, wu_v[...], preferred_element_type=f32)
        gu = (gate * up).astype(bf16)
        whole(WD).wait()
        y = jnp.dot(gu, wd_v[...], preferred_element_type=f32)[:B] * jax.nn.sigmoid(r)
        o_ref[...] = (h + (hn + (hn * 0.0 + y))).astype(o_ref.dtype)

    kt = jnp.transpose(A_k_cache, (0, 1, 3, 2)).reshape(B * H * DH, S)
    vt = jnp.transpose(A_v_cache, (0, 1, 3, 2)).reshape(B * H * DH, S)
    out = pl.pallas_call(
        kernel,
        in_specs=[pl.BlockSpec(memory_space=pl.ANY)] * 9,
        out_specs=pl.BlockSpec(memory_space=pltpu.VMEM),
        out_shape=jax.ShapeDtypeStruct((B, D), A_x.dtype),
        scratch_shapes=[
            pltpu.VMEM((_NBUF, NJ, PR, SC), bf16),
            pltpu.VMEM((B, D), bf16),
            pltpu.VMEM((D,), bf16),
            pltpu.VMEM((D, H * DH), bf16),
            pltpu.VMEM((H * DH, D), bf16),
            pltpu.VMEM((D, F), bf16),
            pltpu.VMEM((D, F), bf16),
            pltpu.VMEM((F, D), bf16),
            pltpu.VMEM((NP, 8, PR), f32),
            pltpu.VMEM((NP, 8, PR), f32),
            pltpu.VMEM((NJ, 8, SC), f32),
            pltpu.SemaphoreType.DMA((_NBUF,)),
            pltpu.SemaphoreType.DMA((7,)),
        ],
        compiler_params=pltpu.CompilerParams(vmem_limit_bytes=64 * 1024 * 1024),
    )(A_x.reshape(B, D), B_w_r, kt, vt, A_wq, A_wo, B_w_gate, B_w_up, B_w_down)
    return out.reshape(B, Sq, D)
```

```python
import jax
import jax.numpy as jnp
from jax import lax
import jax.experimental.pallas as pl
import jax.experimental.pallas.tpu as pltpu

_NBUF = 3
_CC = 256
_CR = (48, 144, 144, 48)
_EPS = 1e-5


def _layernorm(x):
    m = jnp.mean(x, axis=-1, keepdims=True)
    xc = x - m
    v = jnp.mean(xc * xc, axis=-1, keepdims=True)
    return xc / jnp.sqrt(v + _EPS)


def _loop(n, fn):
    def body(j, carry):
        fn(j)
        return carry
    lax.fori_loop(0, n, body, 0)


@jax.jit
def pallas_sequential_preLN__mha_block_cached__moe_arch_mod__decode_kernel(
    A_x: jax.Array,
    A_k_cache: jax.Array,
    A_v_cache: jax.Array,
    A_wq: jax.Array,
    A_wo: jax.Array,
    B_x: jax.Array,
    B_w_r: jax.Array,
    B_w_gate: jax.Array,
    B_w_up: jax.Array,
    B_w_down: jax.Array,
):
    del B_x
    B, Sq, D = A_x.shape
    _, H, S, DH = A_k_cache.shape
    F = B_w_gate.shape[1]
    PR = 2 * DH
    NP = H // 2
    SC = 2 * _CC
    NJ = S // SC
    NF = F // PR
    assert Sq == 1 and B <= 8 and NJ == NP and 3 * NF <= NJ and sum(_CR) == PR
    bf16, f32 = jnp.bfloat16, jnp.float32

    def kernel(x_hbm, wr_hbm, k_hbm, v_hbm, wq_hbm, wo_hbm, wg_hbm, wu_hbm, wd_hbm, o_ref,
               kv, x_v, wr_v, wq_v, wo_v, wg_v, wu_v, wd_v, q_s, o_s, s_s,
               kv_sems, w_sems, wd_sems):
        WQ, WO, WG, WU, X, WR, WD = range(7)
        pairs = ((wq_hbm, wq_v), (wo_hbm, wo_v), (wg_hbm, wg_v), (wu_hbm, wu_v),
                 (x_hbm, x_v), (wr_hbm, wr_v), (wd_hbm, wd_v))

        def start_kv(src, pair, slot, j):
            r0 = pl.multiple_of(pair * PR, PR)
            c0 = pl.multiple_of(j * SC, SC)
            r = 0
            for n in _CR:
                for t in range(2):
                    pltpu.make_async_copy(
                        src.at[pl.ds(r0 + r, n), pl.ds(c0 + t * _CC, _CC)],
                        kv.at[slot, j, pl.ds(r, n), pl.ds(t * _CC, _CC)],
                        kv_sems.at[slot]).start(priority=t)
                r += n

        def wait_kv(slot):
            pltpu.make_async_copy(kv.at[slot], kv.at[slot], kv_sems.at[slot]).wait()

        def whole(i):
            return pltpu.make_async_copy(pairs[i][0], pairs[i][1], w_sems.at[i])

        def start_pieces(i, pieces, sem):
            for n, sl in enumerate(pieces):
                pltpu.make_async_copy(pairs[i][0].at[sl], pairs[i][1].at[sl],
                                      sem).start(priority=n % 2)

        def start_cols(i, g):
            c0 = pl.multiple_of(g * PR, PR)
            start_pieces(i, [(pl.ds(r, 64), pl.ds(c0, PR)) for r in range(0, D, 64)],
                         w_sems.at[i])

        def start_rows(i, g, n, sem):
            r0 = pl.multiple_of(g * PR, PR)
            start_pieces(i, [pl.ds(r0 + r, n) for r in range(0, PR, n)], sem)

        def pad8(a):
            return jnp.concatenate([a, jnp.zeros((8 - B, D), a.dtype)], axis=0)

        whole(X).start()
        whole(WR).start(priority=1)
        _loop(NP, lambda g: start_cols(WQ, g))
        _loop(NJ, lambda j: start_kv(k_hbm, 0, 0, j))
        whole(X).wait()
        whole(WR).wait()
        xn = pad8(_layernorm(x_v[...].astype(f32)).astype(bf16))
        o_s[...] = jnp.zeros(o_s.shape, f32)
        whole(WQ).wait()

        def q_step(g):
            start_kv(v_hbm, 0, 1, g)
            w = wq_v[:, pl.ds(pl.multiple_of(g * PR, PR), PR)]
            q_s[g] = jnp.dot(xn, w, preferred_element_type=f32)
        _loop(NP, q_step)

        row = lax.broadcasted_iota(jnp.int32, (8, PR), 0)
        col = lax.broadcasted_iota(jnp.int32, (8, PR), 1)
        own = jnp.logical_or(jnp.logical_and(row == 0, col < DH),
                             jnp.logical_and(row == 1, col >= DH))
        scale = DH ** -0.5

        def attend(p, issue_in_qk, issue_in_pv):
            b, hp = p // NP, p % NP
            ks, vs = (2 * p) % _NBUF, (2 * p + 1) % _NBUF
            q = jnp.broadcast_to(q_s[hp, pl.ds(b, 1), :], (8, PR))
            q = jnp.where(own, q, 0.0).astype(bf16)

            def qk(j, m):
                issue_in_qk(j)
                s = jnp.dot(q, kv[ks, j], preferred_element_type=f32) * scale
                s_s[j] = s
                return jnp.maximum(m, s)

            wait_kv(ks)
            m = lax.fori_loop(0, NJ, qk, jnp.full((8, SC), -jnp.inf, f32))
            m = jnp.max(m, axis=-1, keepdims=True)

            def pv(j, carry):
                acc, l = carry
                issue_in_pv(j)
                e = jnp.exp(s_s[j] - m)
                acc = acc + lax.dot_general(e.astype(bf16), kv[vs, j], (((1,), (1,)), ((), ())),
                                            preferred_element_type=f32)
                return acc, l + e

            wait_kv(vs)
            acc, l = lax.fori_loop(0, NJ, pv, (jnp.zeros((8, PR), f32), jnp.zeros((8, SC), f32)))
            o = jnp.where(own, acc / jnp.sum(l, axis=-1, keepdims=True), 0.0)
            o_s[hp, pl.ds(b, 1), :] = jnp.sum(o, axis=0, keepdims=True)

        _loop(B * NP - 1, lambda p: attend(
            p,
            lambda j: start_kv(k_hbm, p + 1, (2 * p + 2) % _NBUF, j),
            lambda j: start_kv(v_hbm, p + 1, (2 * p + 3) % _NBUF, j)))

        def start_ffn(j):
            pl.when(j < NF)(lambda: start_cols(WG, j))
            pl.when(jnp.logical_and(j >= NF, j < 2 * NF))(lambda: start_cols(WU, j - NF))
            pl.when(jnp.logical_and(j >= 2 * NF, j < 3 * NF))(
                lambda: start_rows(WD, j - 2 * NF, DH, wd_sems.at[j - 2 * NF]))

        attend(B * NP - 1, lambda j: start_rows(WO, j, 48, w_sems.at[WO]), start_ffn)

        whole(WO).wait()
        attn = jnp.zeros((8, D), f32)
        for g in range(NP):
            attn = attn + jnp.dot(o_s[g].astype(bf16), wo_v[g * PR:(g + 1) * PR, :],
                                  preferred_element_type=f32)
        h = x_v[...].astype(f32) + attn[:B]
        hn = _layernorm(h)
        r = jnp.sum(hn * wr_v[...].astype(f32).reshape(1, D), axis=-1, keepdims=True)
        hb = pad8(hn.astype(bf16))
        whole(WG).wait()
        gate = jnp.dot(hb, wg_v[...], preferred_element_type=f32)
        gate = gate * jax.nn.sigmoid(gate)
        whole(WU).wait()
        up = jnp.dot(hb, wu_v[...], preferred_element_type=f32)
        gu = (gate * up).astype(bf16)
        y = jnp.zeros((8, D), f32)
        for g in range(NF):
            rows = pl.ds(g * PR, PR)
            pltpu.make_async_copy(wd_hbm.at[rows], wd_v.at[rows], wd_sems.at[g]).wait()
            y = y + jnp.dot(gu[:, g * PR:(g + 1) * PR], wd_v[rows, :],
                            preferred_element_type=f32)
        y = y[:B] * jax.nn.sigmoid(r)
        o_ref[...] = (h + (hn + (hn * 0.0 + y))).astype(o_ref.dtype)

    kt = jnp.transpose(A_k_cache, (0, 1, 3, 2)).reshape(B * H * DH, S)
    vt = jnp.transpose(A_v_cache, (0, 1, 3, 2)).reshape(B * H * DH, S)
    out = pl.pallas_call(
        kernel,
        in_specs=[pl.BlockSpec(memory_space=pl.ANY)] * 9,
        out_specs=pl.BlockSpec(memory_space=pltpu.VMEM),
        out_shape=jax.ShapeDtypeStruct((B, D), A_x.dtype),
        scratch_shapes=[
            pltpu.VMEM((_NBUF, NJ, PR, SC), bf16),
            pltpu.VMEM((B, D), bf16),
            pltpu.VMEM((D,), bf16),
            pltpu.VMEM((D, H * DH), bf16),
            pltpu.VMEM((H * DH, D), bf16),
            pltpu.VMEM((D, F), bf16),
            pltpu.VMEM((D, F), bf16),
            pltpu.VMEM((F, D), bf16),
            pltpu.VMEM((NP, 8, PR), f32),
            pltpu.VMEM((NP, 8, PR), f32),
            pltpu.VMEM((NJ, 8, SC), f32),
            pltpu.SemaphoreType.DMA((_NBUF,)),
            pltpu.SemaphoreType.DMA((6,)),
            pltpu.SemaphoreType.DMA((NF,)),
        ],
        compiler_params=pltpu.CompilerParams(vmem_limit_bytes=64 * 1024 * 1024),
    )(A_x.reshape(B, D), B_w_r, kt, vt, A_wq, A_wo, B_w_gate, B_w_up, B_w_down)
    return out.reshape(B, Sq, D)
```
